```python
import jax
import jax.numpy as jnp

def _softmax(x, axis=-1):
    return jax.nn.softmax(x, axis=axis)

def _gelu(x):
    return jax.nn.gelu(x, approximate=True)

def _silu(x):
    return jax.nn.silu(x)

def _sigmoid(x):
    return jax.nn.sigmoid(x)

def _layernorm(x, axis=-1, eps=1e-05):
    m = jnp.mean(x, axis=axis, keepdims=True)
    v = jnp.var(x, axis=axis, keepdims=True)
    return (x - m) / jnp.sqrt(v + eps)

def _scatter_add(tgt, idx, src, axis=0):
    return tgt.at[idx].add(src)

def _segment_sum(src, seg, n):
    return jax.ops.segment_sum(src, seg, n)

class _Rng:

    def __init__(self, key):
        self._k = key

    def _next(self):
        self._k, sub = jax.random.split(self._k)
        return sub

    def normal(self, shape):
        return jax.random.normal(self._next(), shape, dtype=jnp.bfloat16)

    def randint(self, lo, hi, shape):
        return jax.random.randint(self._next(), shape, lo, hi, dtype=jnp.int32)

    def uniform(self, shape, lo=0.0, hi=1.0):
        return jax.random.uniform(self._next(), shape, jnp.bfloat16, lo, hi)

    def permutation(self, n):
        return jax.random.permutation(self._next(), n)
kernel_name = 'recurrent_scan__memory_aug_recurrent_mem_tr__moe_arch_mod__prompt'

def setup_inputs():
    _rng = _Rng(jax.random.key(int.from_bytes(__import__("os").urandom(4), "little")))
    _w = lambda a: (lambda t: t.astype(jnp.bfloat16) if jnp.issubdtype(t.dtype, jnp.floating) else t)(jnp.asarray(a))

    def _A_setup():
        B, S, Dm = (1, 2048, 640)
        H, Dh = (32, 128)
        M, seg = (8, 32)
        seg = min(seg, S)
        S = S // seg * seg
        return {'x': _w((lambda *s: _rng.normal(s) * 0.05)(B, S, Dm)), 'mem0': _w((lambda *s: _rng.normal(s) * 0.05)(B, M, Dm)), 'Wq': _w((lambda *s: _rng.normal(s) * 0.05)(Dm, H, Dh) * Dm ** (-0.5)), 'Wk': _w((lambda *s: _rng.normal(s) * 0.05)(Dm, H, Dh) * Dm ** (-0.5)), 'Wv': _w((lambda *s: _rng.normal(s) * 0.05)(Dm, H, Dh) * Dm ** (-0.5)), 'Wo': _w((lambda *s: _rng.normal(s) * 0.05)(H, Dh, Dm) * (H * Dh) ** (-0.5)), 'seg_len': seg}
    _A_in = _A_setup()

    def _B_setup():
        B, S, D, F, C = (1, 2048, 640, 1728, 8)
        return {'x': _w((lambda *s: _rng.normal(s) * 0.05)(B, S, D)), 'w_r': _w((lambda *s: _rng.normal(s) * 0.05)(D)), 'w_gate': _w((lambda *s: _rng.normal(s) * 0.05)(D, F)), 'w_up': _w((lambda *s: _rng.normal(s) * 0.05)(D, F)), 'w_down': _w((lambda *s: _rng.normal(s) * 0.05)(F, D))}
    _B_in = _B_setup()
    return {'A_x': _A_in['x'], 'A_mem0': _A_in['mem0'], 'A_Wq': _A_in['Wq'], 'A_Wk': _A_in['Wk'], 'A_Wv': _A_in['Wv'], 'A_Wo': _A_in['Wo'], 'A_seg_len': _A_in['seg_len'], 'B_x': _B_in['x'], 'B_w_r': _B_in['w_r'], 'B_w_gate': _B_in['w_gate'], 'B_w_up': _B_in['w_up'], 'B_w_down': _B_in['w_down']}

def reference(A_x, A_mem0, A_Wq, A_Wk, A_Wv, A_Wo, A_seg_len, B_x, B_w_r, B_w_gate, B_w_up, B_w_down):

    def _A_ref(x, mem0, Wq, Wk, Wv, Wo, seg_len):
        B, S, Dm = x.shape
        H, Dh = (Wq.shape[1], Wq.shape[2])
        M = mem0.shape[1]
        scale = Dh ** (-0.5)
        n_seg = S // seg_len
        L = M + seg_len
        idx = jnp.arange(L)
        mask = (idx[:, None] < M) | (idx[:, None] >= idx[None, :])
        mem = mem0
        outs = []
        for s in range(n_seg):
            xs = x[:, s * seg_len:(s + 1) * seg_len, :].copy()
            h = jnp.concatenate([mem, xs], axis=1)
            q = jnp.einsum('btd,dhe->bhte', h, Wq)
            k = jnp.einsum('btd,dhe->bhte', h, Wk)
            v = jnp.einsum('btd,dhe->bhte', h, Wv)
            scores = jnp.einsum('bhqe,bhke->bhqk', q, k) * scale
            scores = jnp.where(mask[None, None], scores, -1000000000.0)
            p = _softmax(scores, axis=-1)
            o = jnp.einsum('bhqk,bhke->bhqe', p, v)
            o = jnp.einsum('bhte,hed->btd', o, Wo)
            mem = o[:, :M, :].copy()
            outs.append(o[:, M:, :])
        return jnp.concatenate(outs, axis=1)

    def _B_ref(x, w_r, w_gate, w_up, w_down):
        B, S, D = x.shape
        C = 8
        r = x @ w_r
        idx = jnp.argsort(-r, axis=-1)[:, :C]
        idx_e = jnp.repeat(idx.reshape(B, C, 1), D, axis=2)
        x_sel = jnp.take_along_axis(x, idx_e, axis=1)
        g = _silu(x_sel @ w_gate)
        u = x_sel @ w_up
        y = g * u @ w_down
        r_sel = _sigmoid(jnp.take_along_axis(r, idx, axis=1))
        y = y * r_sel.reshape(B, C, 1)
        b_off = (jnp.arange(B) * S).reshape(B, 1)
        flat_idx = (idx + b_off).reshape(B * C)
        zero = (x * 0.0).reshape(B * S, D)
        upd = _scatter_add(zero, flat_idx, y.reshape(B * C, D), axis=0)
        return x + upd.reshape(B, S, D)
    x = A_x
    xn = _layernorm(x, axis=-1)
    s = _A_ref(xn, A_mem0, A_Wq, A_Wk, A_Wv, A_Wo, A_seg_len)
    g = _silu(_B_ref(xn, B_w_r, B_w_gate, B_w_up, B_w_down))
    return x + s * g
```

```python
import functools

import jax
import jax.numpy as jnp
import numpy as np
import jax.experimental.pallas as pl
import jax.experimental.pallas.tpu as pltpu

F32 = jnp.float32
BF16 = jnp.bfloat16
U32 = jnp.uint32

_TOPK = 8
_LN_EPS = 1e-5
_NEG = -1000000000.0
_HG = 4
_LN_ROWS = 128
_NT = (((1,), (1,)), ((), ()))


def _rb(v):
    return v.astype(BF16).astype(F32)


def _silu(v):
    return v * (1.0 / (1.0 + jnp.exp(-v)))


def _kernel(x_hbm, mem0_ref, wq_hbm, wk_hbm, wv_hbm, wo_hbm, wr_ref, wg_hbm, wu_hbm, wd_hbm,
            out_hbm,
            x_v, xn_v, gate_v, r_v, raw_q, raw_k, raw_v, wq32, wk32, wv32, wo_v,
            wg_v, wu_v, wd_v, h_v, o_v, out_v, sems, out_sem,
            *, seg, n_heads):
    S, D = x_v.shape
    M = mem0_ref.shape[0]
    L = M + seg
    n_seg = S // seg
    Dh = wq32.shape[2]
    n_grp = n_heads // _HG
    n_dt = D // 128
    scale = float(Dh) ** -0.5

    cp_x = pltpu.make_async_copy(x_hbm, x_v, sems.at[0])
    cp_q = pltpu.make_async_copy(wq_hbm.bitcast(U32), raw_q, sems.at[1])
    cp_k = pltpu.make_async_copy(wk_hbm.bitcast(U32), raw_k, sems.at[2])
    cp_v = pltpu.make_async_copy(wv_hbm.bitcast(U32), raw_v, sems.at[3])
    cp_o = [pltpu.make_async_copy(wo_hbm.at[:, pl.ds(j * 128, 128)], wo_v.at[j], sems.at[4 + j])
            for j in range(n_dt)]
    cp_g = pltpu.make_async_copy(wg_hbm, wg_v, sems.at[4 + n_dt])
    cp_u = pltpu.make_async_copy(wu_hbm, wu_v, sems.at[5 + n_dt])
    cp_d = pltpu.make_async_copy(wd_hbm, wd_v, sems.at[6 + n_dt])
    for cp in [cp_x, cp_g, cp_u, cp_d, cp_q, cp_k, cp_v] + cp_o:
        cp.start()

    cp_x.wait()
    wr = wr_ref[...].astype(F32).reshape(1, D)
    eps = float(np.asarray(_LN_EPS, dtype=jnp.bfloat16).astype(np.float32))
    lane = jax.lax.broadcasted_iota(jnp.int32, (8, 128), 1)
    blk_per_chunk = _LN_ROWS // 8
    chunks_per_vreg = 128 // blk_per_chunk

    def ln_chunk(c, racc):
        rows = pl.ds(pl.multiple_of(c * _LN_ROWS, _LN_ROWS), _LN_ROWS)
        x32 = x_v[rows, :].astype(F32)
        mean = jnp.sum(x32, axis=-1, keepdims=True) / float(D)
        cen = x32 - mean
        var = jnp.sum(cen * cen, axis=-1, keepdims=True) / float(D)
        sd = _rb(jnp.sqrt(_rb(_rb(var) + eps)))
        xn = _rb(_rb(x32 - _rb(mean)) / sd)
        xn_v[rows, :] = xn
        gate_v[rows, :] = _silu(xn)
        r = _rb(jnp.sum(xn * wr, axis=-1, keepdims=True))
        base = (c % chunks_per_vreg) * blk_per_chunk
        for b in range(blk_per_chunk):
            racc = jnp.where(lane == base + b, r[b * 8:(b + 1) * 8, :], racc)
        return racc

    n_rv = S // (8 * 128)
    for j in range(n_rv):
        racc = jax.lax.fori_loop(j * chunks_per_vreg, (j + 1) * chunks_per_vreg, ln_chunk,
                                 jnp.zeros((8, 128), F32))
        r_v[:, j * 128:(j + 1) * 128] = racc

    rr = r_v[...]
    tok = (jax.lax.broadcasted_iota(jnp.int32, rr.shape, 1) * 8
           + jax.lax.broadcasted_iota(jnp.int32, rr.shape, 0))
    sub = jax.lax.broadcasted_iota(jnp.int32, (_TOPK, 1), 0)
    r_sel = jnp.zeros((_TOPK, 1), F32)
    idxs = []
    for i in range(_TOPK):
        m = jnp.max(jnp.max(rr, axis=1, keepdims=True), axis=0, keepdims=True)
        cand = jnp.where(rr == m, tok, S - 1)
        iv = jnp.min(jnp.min(cand, axis=1, keepdims=True), axis=0, keepdims=True)
        rr = jnp.where(tok == iv, -jnp.inf, rr)
        r_sel = jnp.where(sub == i, m, r_sel)
        idxs.append(jnp.clip(jnp.min(iv), 0, S - 1))
    x_sel = jnp.concatenate([xn_v[pl.ds(ix, 1), :] for ix in idxs], axis=0)

    cp_g.wait()
    cp_u.wait()
    cp_d.wait()
    gp = _rb(jax.lax.dot_general(x_sel, wg_v[...], _NT, preferred_element_type=F32))
    up = _rb(jax.lax.dot_general(x_sel, wu_v[...], _NT, preferred_element_type=F32))
    gu = _rb(_rb(_silu(gp)) * up)
    y = _rb(jnp.dot(gu, wd_v[...], preferred_element_type=F32))
    y = _rb(y * _rb(1.0 / (1.0 + jnp.exp(-r_sel))))
    g_sel = _silu(_rb(x_sel + y))
    for i, ix in enumerate(idxs):
        gate_v[pl.ds(ix, 1), :] = g_sel[i:i + 1, :]

    def repack(raw, dst):
        n_pair = n_heads // 2

        def body(j, c):
            a = raw[pl.ds(j, D, stride=n_pair), :]
            lo = pltpu.bitcast(a << 16, F32).astype(BF16)
            hi = pltpu.bitcast(a & np.uint32(0xFFFF0000), F32).astype(BF16)
            dst[2 * j] = pltpu.bitcast(lo, U32)
            dst[2 * j + 1] = pltpu.bitcast(hi, U32)
            return c
        jax.lax.fori_loop(0, n_pair, body, 0)

    cp_q.wait()
    repack(raw_q, wq32)
    cp_k.wait()
    repack(raw_k, wk32)
    cp_v.wait()
    repack(raw_v, wv32)
    for cp in cp_o:
        cp.wait()
    wo32 = wo_v.bitcast(U32)

    h_v[0:M, :] = mem0_ref[...].astype(F32)

    def out_copy(s):
        rows = pl.ds(pl.multiple_of(s * seg, seg), seg)
        return pltpu.make_async_copy(out_v.at[rows, :], out_hbm.at[rows, :], out_sem.at[0])

    def step(s, carry):
        rows = pl.ds(pl.multiple_of(s * seg, seg), seg)
        h_v[M:L, :] = xn_v[rows, :]
        ri = jax.lax.broadcasted_iota(jnp.int32, (L, L), 0)
        ci = jax.lax.broadcasted_iota(jnp.int32, (L, L), 1)
        mask = (ri < M) | (ri >= ci)

        def proj(w32, g):
            w = jnp.concatenate([pltpu.bitcast(w32[g * _HG + i], BF16) for i in range(_HG)], axis=1)
            return jnp.dot(h_v[...], w, preferred_element_type=F32)

        def probs(q, k):
            ps = []
            for i in range(_HG):
                sl = slice(i * Dh, (i + 1) * Dh)
                sc = jax.lax.dot_general(q[:, sl], k[:, sl], _NT, preferred_element_type=F32)
                sc = jnp.where(mask, sc * scale, _NEG)
                e = jnp.exp(sc - jnp.max(sc, axis=-1, keepdims=True))
                lsum = jnp.sum(e, axis=-1, keepdims=True)
                rc = pl.reciprocal(lsum, approx=True)
                rc = rc * (2.0 - lsum * rc)
                ps.append(e * rc)
            return ps

        def pv(ps, v, g):
            for i in range(_HG):
                sl = slice(i * Dh, (i + 1) * Dh)
                hh = g * _HG + i
                o_v[:, hh * Dh:(hh + 1) * Dh] = jnp.dot(ps[i], v[:, sl], preferred_element_type=F32)

        def oproj(g0, g1):
            k0, k1 = g0 * _HG * Dh, g1 * _HG * Dh
            w = jnp.concatenate([pltpu.bitcast(wo32[j, k0 // 2:k1 // 2, :], BF16)
                                 for j in range(n_dt)], axis=1)
            return jnp.dot(o_v[:, k0:k1], w, preferred_element_type=F32)

        q, k, v, p = {}, {}, {}, {}
        for g in range(n_grp):
            q[g] = proj(wq32, g)
            if g > 0:
                p[g - 1] = probs(q[g - 1], k[g - 1])
            k[g] = proj(wk32, g)
            v[g] = proj(wv32, g)
            if g == n_grp - 1:
                p[g] = probs(q[g], k[g])
            if g > 0:
                pv(p[g - 1], v[g - 1], g - 1)
        acc = oproj(0, 2)
        pv(p[n_grp - 1], v[n_grp - 1], n_grp - 1)
        acc = acc + oproj(2, n_grp)

        h_v[0:M, :] = _rb(acc[0:M, :])
        res = x_v[rows, :].astype(F32) + acc[M:L, :] * gate_v[rows, :]
        out_v[rows, :] = res.astype(out_v.dtype)
        out_copy(s).start()
        return carry

    jax.lax.fori_loop(0, n_seg, step, 0)

    def drain(s, c):
        out_copy(s).wait()
        return c
    jax.lax.fori_loop(0, n_seg, drain, 0)


@functools.partial(jax.jit, static_argnames=("A_seg_len",))
def pallas_recurrent_scan__memory_aug_recurrent_mem_tr__moe_arch_mod__prompt_kernel(
    A_x: jax.Array,
    A_mem0: jax.Array,
    A_Wq: jax.Array,
    A_Wk: jax.Array,
    A_Wv: jax.Array,
    A_Wo: jax.Array,
    A_seg_len: int,
    B_x: jax.Array,
    B_w_r: jax.Array,
    B_w_gate: jax.Array,
    B_w_up: jax.Array,
    B_w_down: jax.Array,
):
    del B_x
    B, S, D = A_x.shape
    _, H, Dh = A_Wq.shape
    M = A_mem0.shape[1]
    Fh = B_w_gate.shape[1]
    seg = int(A_seg_len)
    assert B == 1 and Dh == 128 and D % 128 == 0 and H % (2 * _HG) == 0
    assert S % seg == 0 and seg % 16 == 0 and M % 8 == 0 and M + seg <= 128 and S % 1024 == 0
    L = M + seg
    n_dt = D // 128

    hbm = pl.BlockSpec(memory_space=pltpu.MemorySpace.HBM)
    vmem = pl.BlockSpec(memory_space=pltpu.VMEM)
    out = pl.pallas_call(
        functools.partial(_kernel, seg=seg, n_heads=H),
        out_shape=jax.ShapeDtypeStruct((S, D), A_x.dtype),
        in_specs=[hbm, vmem, hbm, hbm, hbm, hbm, vmem, hbm, hbm, hbm],
        out_specs=hbm,
        scratch_shapes=[
            pltpu.VMEM((S, D), A_x.dtype),
            pltpu.VMEM((S, D), F32),
            pltpu.VMEM((S, D), F32),
            pltpu.VMEM((8, S // 8), F32),
            pltpu.VMEM((D * H // 2, Dh), U32),
            pltpu.VMEM((D * H // 2, Dh), U32),
            pltpu.VMEM((D * H // 2, Dh), U32),
            pltpu.VMEM((H, D // 2, Dh), U32),
            pltpu.VMEM((H, D // 2, Dh), U32),
            pltpu.VMEM((H, D // 2, Dh), U32),
            pltpu.VMEM((n_dt, H * Dh, 128), BF16),
            pltpu.VMEM((Fh, D), BF16),
            pltpu.VMEM((Fh, D), BF16),
            pltpu.VMEM((Fh, D), BF16),
            pltpu.VMEM((L, D), F32),
            pltpu.VMEM((L, H * Dh), F32),
            pltpu.VMEM((S, D), A_x.dtype),
            pltpu.SemaphoreType.DMA((7 + n_dt,)),
            pltpu.SemaphoreType.DMA((1,)),
        ],
        compiler_params=pltpu.CompilerParams(vmem_limit_bytes=110 * 1024 * 1024),
        name="rmt_moe_scan",
    )(
        A_x.reshape(S, D),
        A_mem0.reshape(M, D),
        A_Wq.reshape(D * H, Dh),
        A_Wk.reshape(D * H, Dh),
        A_Wv.reshape(D * H, Dh),
        A_Wo.reshape(H * Dh, D),
        B_w_r,
        B_w_gate.T,
        B_w_up.T,
        B_w_down,
    )
    return out.reshape(B, S, D)
```

```python
import functools

import jax
import jax.numpy as jnp
import numpy as np
import jax.experimental.pallas as pl
import jax.experimental.pallas.tpu as pltpu

F32 = jnp.float32
BF16 = jnp.bfloat16
U32 = jnp.uint32

_TOPK = 8
_LN_EPS = 1e-5
_NEG = -1000000000.0
_HG = 4
_HC = 16
_NT = (((1,), (1,)), ((), ()))

CFG = dict(order="K0 Q0 K1 Q1 S0 V0 K2 Q2 S1 V1 P0 K3 Q3 S2 V2 P1 C0-1 K4 Q4 S3 V3 P2 C1-2 K5 Q5 S4 V4 P3 C2-3 K6 Q6 S5 V5 P4 C3-4 K7 Q7 S6 V6 S7 P5 C4-5 V7 P6 C5-6 P7 C6-7 C7-8", nsteps=None, unroll=1)


def _order(name, n):
    ops = []
    if name == "lag1":
        for g in range(n):
            ops.append(("Q", g))
            if g > 0:
                ops.append(("S", g - 1))
            ops += [("K", g), ("V", g)]
            if g == n - 1:
                ops.append(("S", g))
            if g > 0:
                ops.append(("P", g - 1))
        ops += [("C", 0, 2), ("P", n - 1), ("C", 2, n)]
    elif name == "vlag2":
        for g in range(n + 2):
            if g < n:
                ops += [("Q", g), ("K", g)]
            if 0 <= g - 1 < n:
                ops.append(("S", g - 1))
            if 0 <= g - 2 < n:
                ops.append(("V", g - 2))
            if 0 <= g - 3 < n:
                ops.append(("P", g - 3))
        ops += [("P", n - 1), ("C", 0, n)]
    else:
        for tok in name.split():
            if tok[0] == "C":
                a, b = tok[1:].split("-")
                ops.append(("C", int(a), int(b)))
            else:
                ops.append((tok[0], int(tok[1:])))
    return ops


def _rb(v):
    return v.astype(BF16).astype(F32)


def _silu(v):
    return v * (1.0 / (1.0 + jnp.exp(-v)))


def _kernel(x_hbm, mem0_ref, wq_hbm, wk_hbm, wv_hbm, wo_hbm, wr_ref, wg_hbm, wu_hbm, wd_hbm,
            out_hbm, *scr, seg, n_heads, lead):
    n_chunk = 3 * n_heads // _HC
    n_grp = n_heads // _HG
    gpc = _HC // _HG
    scr = list(scr)
    x_v, xa_v, xb_v, z_v, wo_v, wg_v, wu_v, wd_v, h_v, o_v, out_v, sems, out_sem = scr[:13]
    raw = scr[13:13 + n_chunk]
    w32 = scr[13 + n_chunk:13 + 2 * n_chunk]
    ring = scr[13 + 2 * n_chunk:]
    S, D = x_v.shape
    M = mem0_ref.shape[0]
    L = M + seg
    n_seg = S // seg
    Dh = w32[0].shape[2]
    n_dt = D // 128
    scale = float(Dh) ** -0.5
    adv = seg - M
    ring_blk = ring[0].shape[0] // 8

    cp_xa = pltpu.make_async_copy(x_hbm.at[0:lead, :], x_v.at[0:lead, :], sems.at[0])
    cp_xb = pltpu.make_async_copy(x_hbm.at[lead:S, :], x_v.at[lead:S, :], sems.at[1])
    cp_w = []
    for c in range(n_chunk):
        src = (wq_hbm, wk_hbm, wv_hbm)[c // (n_heads // _HC)].bitcast(U32)
        j0 = (c % (n_heads // _HC)) * (_HC // 2)
        cp_w.append(pltpu.make_async_copy(src.at[:, pl.ds(j0, _HC // 2), :],
                                          raw[c].reshape(D, _HC // 2, Dh), sems.at[2 + c]))
    nb = 2 + n_chunk
    cp_o = [pltpu.make_async_copy(wo_hbm.at[:, pl.ds(j * 128, 128)], wo_v.at[j], sems.at[nb + j])
            for j in range(n_dt)]
    cp_g = pltpu.make_async_copy(wg_hbm, wg_v, sems.at[nb + n_dt])
    cp_u = pltpu.make_async_copy(wu_hbm, wu_v, sems.at[nb + n_dt + 1])
    cp_d = pltpu.make_async_copy(wd_hbm, wd_v, sems.at[nb + n_dt + 2])
    SKIP = CFG.get("skip_pro")
    if not SKIP:
        for cp in [cp_xa, cp_w[0], cp_w[1], cp_xb] + cp_w[2:] + [cp_g, cp_u, cp_d] + cp_o:
            cp.start()

    wr = wr_ref[...].astype(F32).reshape(1, D)
    eps = float(np.asarray(_LN_EPS, dtype=jnp.bfloat16).astype(np.float32))
    lane = jax.lax.broadcasted_iota(jnp.int32, (8, 128), 1)
    n_rv = S // (8 * 128)

    def ln_rows(row0, nrows, dst, dst0, racc):
        rows = pl.ds(row0, nrows)
        x32 = x_v[rows, :].astype(F32)
        mean = jnp.sum(x32, axis=-1, keepdims=True) * (1.0 / D)
        cen = x32 - mean
        var = jnp.sum(cen * cen, axis=-1, keepdims=True) * (1.0 / D)
        sd = _rb(jnp.sqrt(_rb(_rb(var) + eps)))
        xn = _rb(_rb(x32 - _rb(mean)) * (1.0 / sd))
        dst[pl.ds(dst0, nrows), :] = xn
        z_v[rows, :] = xn
        r = _rb(jnp.sum(xn * wr, axis=-1, keepdims=True))
        racc = list(racc)
        for b in range(nrows // 8):
            blk = row0 // 8 + b
            for j in range(n_rv):
                racc[j] = jnp.where(lane == blk - j * 128, r[b * 8:(b + 1) * 8, :], racc[j])
        return tuple(racc)

    def repack(c, j, d0, nd):
        pairs = _HC // 2
        a = raw[c][pl.ds(d0 * pairs + j, nd, stride=pairs), :]
        lo = pltpu.bitcast(a << 16, F32).astype(BF16)
        hi = pltpu.bitcast(a & np.uint32(0xFFFF0000), F32).astype(BF16)
        w32[c][2 * j, d0 // 2:(d0 + nd) // 2, :] = pltpu.bitcast(lo, U32)
        w32[c][2 * j + 1, d0 // 2:(d0 + nd) // 2, :] = pltpu.bitcast(hi, U32)

    def weights(m, g):
        c, h0 = (m * n_grp + g) // gpc, ((m * n_grp + g) % gpc) * _HG
        return jnp.concatenate([pltpu.bitcast(w32[c][h0 + i], BF16) for i in range(_HG)], axis=1)

    if not SKIP:
        cp_xa.wait()
        racc = tuple(jnp.zeros((8, 128), F32) for _ in range(n_rv))
        pr = 128
        n_pb = lead // pr
        racc = jax.lax.fori_loop(
            0, n_pb,
            lambda i, c: ln_rows(pl.multiple_of(i * pr, pr), pr, xa_v, pl.multiple_of(i * pr, pr), c),
            racc)
        cp_w[0].wait()

        def repack_all(j, c):
            repack(0, j, 0, D)
            return c
        jax.lax.fori_loop(0, _HC // 2, repack_all, 0)

        ln_phases = 4
        ln_per = (S - lead) // (ln_phases * n_pb)
        ppb = (_HC // 2) // n_pb

        def routing(racc):
            rr = jnp.concatenate(racc, axis=1)
            tok = (jax.lax.broadcasted_iota(jnp.int32, rr.shape, 1) * 8
                   + jax.lax.broadcasted_iota(jnp.int32, rr.shape, 0))
            sub = jax.lax.broadcasted_iota(jnp.int32, (_TOPK, 1), 0)
            r_sel = jnp.zeros((_TOPK, 1), F32)
            idxs = []
            for i in range(_TOPK):
                m = jnp.max(jnp.max(rr, axis=1, keepdims=True), axis=0, keepdims=True)
                cand = jnp.where(rr == m, tok, S - 1)
                iv = jnp.min(jnp.min(cand, axis=1, keepdims=True), axis=0, keepdims=True)
                rr = jnp.where(tok == iv, -jnp.inf, rr)
                r_sel = jnp.where(sub == i, m, r_sel)
                idxs.append(jnp.clip(jnp.min(iv), 0, S - 1))
            return idxs, r_sel, jnp.concatenate([z_v[pl.ds(ix, 1), :] for ix in idxs], axis=0)

        def expert(idxs, r_sel, x_sel):
            gp = _rb(jax.lax.dot_general(x_sel, wg_v[...], _NT, preferred_element_type=F32))
            up = _rb(jax.lax.dot_general(x_sel, wu_v[...], _NT, preferred_element_type=F32))
            gu = _rb(_rb(_silu(gp)) * up)
            y = _rb(jnp.dot(gu, wd_v[...], preferred_element_type=F32))
            y = _rb(y * _rb(1.0 / (1.0 + jnp.exp(-r_sel))))
            z_sel = _rb(x_sel + y)
            for i, ix in enumerate(idxs):
                z_v[pl.ds(ix, 1), :] = z_sel[i:i + 1, :]

        def block(i, racc, c, pair0, npair, ln):
            rows = pl.ds(pl.multiple_of(i * pr, pr), pr)
            for gg in range(gpc):
                mg = c * gpc + gg
                ring[mg][rows, :] = jnp.dot(xa_v[rows, :], weights(mg // n_grp, mg % n_grp),
                                            preferred_element_type=F32)
                if npair:
                    pieces = npair * 2 // gpc
                    for pc in range(gg * pieces, (gg + 1) * pieces):
                        repack(c + 1, pair0(i) + pc // 2, (pc % 2) * (D // 2), D // 2)
                if ln and gg < ln_per // 32:
                    off = pl.multiple_of(((c - 1) * n_pb + i) * ln_per + gg * 32, 32)
                    racc = ln_rows(lead + off, 32, xb_v, off, racc)
            return racc

        half = n_pb // 2
        racc = jax.lax.fori_loop(0, half, functools.partial(block, c=0, pair0=None, npair=0, ln=False), racc)
        cp_w[1].wait()
        racc = jax.lax.fori_loop(half, n_pb, functools.partial(
            block, c=0, pair0=lambda i: (i - half) * 2 * ppb, npair=2 * ppb, ln=False), racc)
        cp_xb.wait()
        for c in range(1, n_chunk - 1):
            cp_w[c + 1].wait()
            racc = jax.lax.fori_loop(0, n_pb, functools.partial(
                block, c=c, pair0=lambda i: i * ppb, npair=ppb, ln=True), racc)
        last = functools.partial(block, c=n_chunk - 1, pair0=None, npair=0, ln=False)
        racc = jax.lax.fori_loop(0, n_pb - 2, last, racc)
        cp_g.wait()
        cp_u.wait()
        cp_d.wait()
        routed = routing(racc)
        last(n_pb - 2, racc)
        expert(*routed)
        last(n_pb - 1, racc)

        for cp in cp_o:
            cp.wait()
    wo32 = wo_v.bitcast(U32)

    h_v[0:M, :] = mem0_ref[...].astype(F32)

    def out_copy(s):
        rows = pl.ds(pl.multiple_of(s * seg, seg), seg)
        return pltpu.make_async_copy(out_v.at[rows, :], out_hbm.at[rows, :], out_sem.at[0])

    def wrap(b):
        return jnp.where(b >= ring_blk, b - ring_blk, b)

    def step(s, carry):
        rd, wr_blk = carry
        rows = pl.ds(pl.multiple_of(s * seg, seg), seg)
        h_v[M:seg, :] = xb_v[pl.ds(pl.multiple_of(s * adv, 8), adv), :]
        ri = jax.lax.broadcasted_iota(jnp.int32, (L, L), 0)
        ci = jax.lax.broadcasted_iota(jnp.int32, (L, L), 1)
        mask = (ri < M) | (ri >= ci)
        wpos = [pl.multiple_of(wrap(wr_blk + i) * 8, 8) for i in range(adv // 8)]
        rpos = pl.multiple_of(rd * 8, seg)

        def proj(m, g):
            y = jnp.dot(h_v[...], weights(m, g), preferred_element_type=F32)
            buf = ring[m * n_grp + g]
            for i, w in enumerate(wpos):
                buf[pl.ds(w, 8), :] = y[M + 8 * i:M + 8 * i + 8, :]
            return y[0:M, :]

        def full(m, g, top):
            return jnp.concatenate([top, ring[m * n_grp + g][pl.ds(rpos, seg), :]], axis=0)

        def probs(q, k):
            ps = []
            for i in range(_HG):
                sl = slice(i * Dh, (i + 1) * Dh)
                sc = jax.lax.dot_general(q[:, sl], k[:, sl], _NT, preferred_element_type=F32)
                sc = jnp.where(mask, sc * scale, _NEG)
                e = jnp.exp(sc - jnp.max(sc, axis=-1, keepdims=True))
                lsum = jnp.sum(e, axis=-1, keepdims=True)
                rc = pl.reciprocal(lsum, approx=True)
                rc = rc * (2.0 - lsum * rc)
                ps.append(e * rc)
            return ps

        def pv(ps, v, g):
            for i in range(_HG):
                sl = slice(i * Dh, (i + 1) * Dh)
                hh = g * _HG + i
                o_v[:, hh * Dh:(hh + 1) * Dh] = jnp.dot(ps[i], v[:, sl], preferred_element_type=F32)

        def oproj(g0, g1):
            k0, k1 = g0 * _HG * Dh, g1 * _HG * Dh
            w = jnp.concatenate([pltpu.bitcast(wo32[j, k0 // 2:k1 // 2, :], BF16)
                                 for j in range(n_dt)], axis=1)
            return jnp.dot(o_v[:, k0:k1], w, preferred_element_type=F32)

        top, p, acc = {}, {}, None
        for op in _order(CFG["order"], n_grp):
            if op[0] in "QKV":
                m = "QKV".index(op[0])
                top[m, op[1]] = proj(m, op[1])
            elif op[0] == "S":
                g = op[1]
                p[g] = probs(full(0, g, top[0, g]), full(1, g, top[1, g]))
            elif op[0] == "P":
                g = op[1]
                pv(p[g], full(2, g, top[2, g]), g)
            else:
                part = oproj(op[1], op[2])
                acc = part if acc is None else acc + part

        h_v[0:M, :] = _rb(acc[0:M, :])
        res = x_v[rows, :].astype(F32) + acc[M:L, :] * _silu(z_v[rows, :])
        out_v[rows, :] = res.astype(out_v.dtype)
        out_copy(s).start()
        return wrap(rd + seg // 8), wrap(wr_blk + adv // 8)

    if CFG["nsteps"]:
        n_seg = CFG["nsteps"]
    jax.lax.fori_loop(0, n_seg, step, (jnp.int32(0), jnp.int32(lead // 8)), unroll=CFG["unroll"])

    def drain(s, c):
        out_copy(s).wait()
        return c
    jax.lax.fori_loop(0, n_seg, drain, 0)


@functools.partial(jax.jit, static_argnames=("A_seg_len",))
def pallas_recurrent_scan__memory_aug_recurrent_mem_tr__moe_arch_mod__prompt_kernel(
    A_x, A_mem0, A_Wq, A_Wk, A_Wv, A_Wo, A_seg_len, B_x, B_w_r, B_w_gate, B_w_up, B_w_down,
):
    del B_x
    B, S, D = A_x.shape
    _, H, Dh = A_Wq.shape
    M = A_mem0.shape[1]
    Fh = B_w_gate.shape[1]
    seg = int(A_seg_len)
    L = M + seg
    n_dt = D // 128
    lead = (S // seg) * M
    n_chunk = 3 * H // _HC
    ring_rows = lead + seg

    hbm = pl.BlockSpec(memory_space=pltpu.MemorySpace.HBM)
    vmem = pl.BlockSpec(memory_space=pltpu.VMEM)
    out = pl.pallas_call(
        functools.partial(_kernel, seg=seg, n_heads=H, lead=lead),
        out_shape=jax.ShapeDtypeStruct((S, D), A_x.dtype),
        in_specs=[hbm, vmem, hbm, hbm, hbm, hbm, vmem, hbm, hbm, hbm],
        out_specs=hbm,
        scratch_shapes=[
            pltpu.VMEM((S, D), A_x.dtype),
            pltpu.VMEM((lead, D), F32),
            pltpu.VMEM((S - lead, D), F32),
            pltpu.VMEM((S, D), F32),
            pltpu.VMEM((n_dt, H * Dh, 128), BF16),
            pltpu.VMEM((Fh, D), BF16),
            pltpu.VMEM((Fh, D), BF16),
            pltpu.VMEM((Fh, D), BF16),
            pltpu.VMEM((seg, D), F32),
            pltpu.VMEM((L, H * Dh), F32),
            pltpu.VMEM((S, D), A_x.dtype),
            pltpu.SemaphoreType.DMA((5 + n_chunk + n_dt,)),
            pltpu.SemaphoreType.DMA((1,)),
        ] + [pltpu.VMEM((D * _HC // 2, Dh), U32)] * n_chunk
          + [pltpu.VMEM((_HC, D // 2, Dh), U32)] * n_chunk
          + [pltpu.VMEM((ring_rows, _HG * Dh), F32)] * (3 * H // _HG),
        compiler_params=pltpu.CompilerParams(vmem_limit_bytes=110 * 1024 * 1024),
        name="rmt_moe_scan",
    )(
        A_x.reshape(S, D),
        A_mem0.reshape(M, D),
        A_Wq,
        A_Wk,
        A_Wv,
        A_Wo.reshape(H * Dh, D),
        B_w_r,
        B_w_gate.T,
        B_w_up.T,
        B_w_down,
    )
    return out.reshape(B, S, D)
```

```python
import functools

import jax
import jax.numpy as jnp
import numpy as np
import jax.experimental.pallas as pl
import jax.experimental.pallas.tpu as pltpu

F32 = jnp.float32
BF16 = jnp.bfloat16
U32 = jnp.uint32

_TOPK = 8
_LN_EPS = 1e-5
_NEG = -1000000000.0
_HG = 4
_HC = 16
_NT = (((1,), (1,)), ((), ()))

CFG = dict(order="K0 Q0 K1 Q1 S0 V0 K2 Q2 S1 V1 P0 K3 Q3 S2 V2 P1 C0-1 K4 Q4 S3 V3 P2 C1-2 K5 Q5 S4 V4 P3 C2-3 K6 Q6 S5 V5 P4 C3-4 K7 Q7 S6 V6 S7 P5 C4-5 V7 P6 C5-6 P7 C6-7 C7-8",
           nsteps=None, unroll=4)


def _order(name):
    ops = []
    for tok in name.split():
        if tok[0] == "C":
            a, b = tok[1:].split("-")
            ops.append(("C", int(a), int(b)))
        else:
            ops.append((tok[0], int(tok[1:])))
    return ops


def _rb(v):
    return v.astype(BF16).astype(F32)


def _silu(v):
    return v * (1.0 / (1.0 + jnp.exp(-v)))


def _kernel(x_hbm, mem0_ref, wq_hbm, wk_hbm, wv_hbm, wo_hbm, wr_ref, wg_hbm, wu_hbm, wd_hbm,
            out_hbm,
            x_v, xa_v, xb_v, z_v, raw, w32, ring, wo_v, wg_v, wu_v, wd_v, h_v, o_v, out_v,
            sems, out_sem, *, seg, n_heads, lead, ln_rows0):
    n_chunk = raw.shape[0]
    n_grp = n_heads // _HG
    gpc = _HC // _HG
    S, D = x_v.shape
    M = mem0_ref.shape[0]
    L = M + seg
    n_seg = S // seg
    Dh = w32.shape[2]
    n_dt = D // 128
    scale = float(Dh) ** -0.5
    adv = seg - M
    ring_blk = ring.shape[1] // 8
    SKIP = CFG.get("skip_pro")

    n_it = 3 * n_grp
    ln_per = (S - ln_rows0) // (n_it - 2)
    xb_it = 2
    xs = ln_rows0 + xb_it * ln_per
    cp_xa = pltpu.make_async_copy(x_hbm.at[0:xs, :], x_v.at[0:xs, :], sems.at[0])
    cp_xb = pltpu.make_async_copy(x_hbm.at[xs:S, :], x_v.at[xs:S, :], sems.at[1])
    cp_w = []
    for c in range(n_chunk):
        src = (wq_hbm, wk_hbm, wv_hbm)[c // (n_heads // _HC)].bitcast(U32)
        j0 = (c % (n_heads // _HC)) * (_HC // 2)
        cp_w.append(pltpu.make_async_copy(src.at[:, pl.ds(j0, _HC // 2), :],
                                          raw.at[c].reshape(D, _HC // 2, Dh), sems.at[2 + c]))
    nb = 2 + n_chunk
    cp_o = [pltpu.make_async_copy(wo_hbm.at[:, pl.ds(j * 128, 128)], wo_v.at[j], sems.at[nb + j])
            for j in range(n_dt)]
    cp_g = pltpu.make_async_copy(wg_hbm, wg_v, sems.at[nb + n_dt])
    cp_u = pltpu.make_async_copy(wu_hbm, wu_v, sems.at[nb + n_dt + 1])
    cp_d = pltpu.make_async_copy(wd_hbm, wd_v, sems.at[nb + n_dt + 2])
    if not SKIP:
        for cp in [cp_xa, cp_w[0], cp_xb] + cp_w[1:] + [cp_g, cp_u, cp_d] + cp_o:
            cp.start()

    wr = wr_ref[...].astype(F32).reshape(1, D)
    eps = float(np.asarray(_LN_EPS, dtype=jnp.bfloat16).astype(np.float32))
    lane = jax.lax.broadcasted_iota(jnp.int32, (8, 128), 1)
    n_rv = S // (8 * 128)

    def ln_rows(row0, nrows, dst, dst0, racc):
        rows = pl.ds(row0, nrows)
        x32 = x_v[rows, :].astype(F32)
        mean = jnp.sum(x32, axis=-1, keepdims=True) * (1.0 / D)
        cen = x32 - mean
        var = jnp.sum(cen * cen, axis=-1, keepdims=True) * (1.0 / D)
        sd = _rb(jnp.sqrt(_rb(_rb(var) + eps)))
        xn = _rb(_rb(x32 - _rb(mean)) * (1.0 / sd))
        dst[pl.ds(dst0, nrows), :] = xn
        z_v[rows, :] = xn
        r = _rb(jnp.sum(xn * wr, axis=-1, keepdims=True))
        racc = list(racc)
        for b in range(nrows // 8):
            blk = row0 // 8 + b
            for j in range(n_rv):
                racc[j] = jnp.where(lane == blk - j * 128, r[b * 8:(b + 1) * 8, :], racc[j])
        return tuple(racc)

    def lead_group(it):
        c = it // gpc
        j0 = (it % gpc) * (_HG // 2)
        cols = []
        for jj in range(_HG // 2):
            a = raw[c, pl.ds(j0 + jj, D, stride=_HC // 2), :]
            for p, half in enumerate((a.astype(jnp.uint16), (a >> 16).astype(jnp.uint16))):
                packed = pltpu.bitcast(half, U32)
                w32[it * _HG + 2 * jj + p] = packed
                cols.append(pltpu.bitcast(packed, BF16))
        w = jnp.concatenate(cols, axis=1)
        sub = CFG.get("psub", lead)
        for r0 in range(0, lead, sub):
            ring[it, r0:r0 + sub, :] = jnp.dot(xa_v[r0:r0 + sub, :], w, preferred_element_type=F32)

    def routing(racc):
        rr = jnp.concatenate(racc, axis=1) + 0.0
        tok = (jax.lax.broadcasted_iota(jnp.int32, rr.shape, 1) * 8
               + jax.lax.broadcasted_iota(jnp.int32, rr.shape, 0))
        bits = pltpu.bitcast(rr, jnp.int32)
        mono = jnp.where(bits < 0, bits ^ 0x7FFFFFFF, bits) >> 16
        key = pltpu.bitcast(0x30000000 + (mono + 32768) * S + (S - 1 - tok), F32)
        sub = jax.lax.broadcasted_iota(jnp.int32, (_TOPK, 1), 0)
        best = jnp.zeros((_TOPK, 1), F32)
        for i in range(_TOPK):
            m = jnp.max(jnp.max(key, axis=1, keepdims=True), axis=0, keepdims=True)
            key = jnp.where(key == m, 0.0, key)
            best = jnp.where(sub == i, m, best)
        kb = pltpu.bitcast(best, jnp.int32) - 0x30000000
        sel_tok = (S - 1) - (kb & (S - 1))
        mono = ((kb >> (S.bit_length() - 1)) - 32768) << 16
        r_sel = pltpu.bitcast(jnp.where(mono < 0, (mono | 0xFFFF) ^ 0x7FFFFFFF, mono), F32)
        idxs = [jnp.clip(jnp.max(jnp.where(sub == i, sel_tok, 0)), 0, S - 1) for i in range(_TOPK)]
        return idxs, r_sel, jnp.concatenate([z_v[pl.ds(ix, 1), :] for ix in idxs], axis=0)

    def expert(idxs, r_sel, x_sel):
        gp = _rb(jax.lax.dot_general(x_sel, wg_v[...], _NT, preferred_element_type=F32))
        up = _rb(jax.lax.dot_general(x_sel, wu_v[...], _NT, preferred_element_type=F32))
        gu = _rb(_rb(_silu(gp)) * up)
        y = _rb(jnp.dot(gu, wd_v[...], preferred_element_type=F32))
        y = _rb(y * _rb(1.0 / (1.0 + jnp.exp(-r_sel))))
        z_sel = _rb(x_sel + y)
        for i, ix in enumerate(idxs):
            z_v[pl.ds(ix, 1), :] = z_sel[i:i + 1, :]

    if not SKIP:
        lnb = 128
        cp_xa.wait()
        racc = tuple(jnp.zeros((8, 128), F32) for _ in range(n_rv))
        racc = jax.lax.fori_loop(
            0, lead // lnb,
            lambda i, c: ln_rows(pl.multiple_of(i * lnb, lnb), lnb, xa_v,
                                 pl.multiple_of(i * lnb, lnb), c), racc)
        for r0 in range(lead, ln_rows0, lnb):
            racc = ln_rows(r0, lnb, xb_v, r0 - lead, racc)

        def lead_step(it, racc):
            @pl.when(it % gpc == 0)
            def _():
                c = it // gpc
                pltpu.make_async_copy(raw.at[c], raw.at[c], sems.at[2 + c]).wait()

            @pl.when(it == xb_it)
            def _():
                cp_xb.wait()

            lead_group(it)
            row0 = pl.multiple_of(ln_rows0 + it * ln_per, ln_per)
            return ln_rows(row0, ln_per, xb_v, pl.multiple_of(row0 - lead, ln_per), racc)

        racc = jax.lax.fori_loop(0, n_it - 2, lead_step, racc)
        cp_g.wait()
        cp_u.wait()
        cp_d.wait()
        routed = routing(racc)
        lead_group(n_it - 2)
        expert(*routed)
        lead_group(n_it - 1)
        for cp in cp_o:
            cp.wait()
    wo32 = wo_v.bitcast(U32)

    h_v[adv:seg, :] = mem0_ref[...].astype(F32)

    def out_copy(s):
        rows = pl.ds(pl.multiple_of(s * seg, seg), seg)
        return pltpu.make_async_copy(out_v.at[rows, :], out_hbm.at[rows, :], out_sem.at[0])

    def wrap(b):
        return jnp.where(b >= ring_blk, b - ring_blk, b)

    def step(s, carry):
        rd, wr_blk = carry
        rows = pl.ds(pl.multiple_of(s * seg, seg), seg)
        h_v[0:adv, :] = xb_v[pl.ds(pl.multiple_of(s * adv, 8), adv), :]
        ri = jax.lax.broadcasted_iota(jnp.int32, (L, L), 0)
        ci = jax.lax.broadcasted_iota(jnp.int32, (L, L), 1)
        mask = (ri < M) | (ri >= ci)
        wpos = [pl.multiple_of(wrap(wr_blk + i) * 8, 8) for i in range(adv // 8)]
        rpos = pl.multiple_of(rd * 8, seg)

        def proj(m, g):
            mg = m * n_grp + g
            w = jnp.concatenate([pltpu.bitcast(w32[mg * _HG + i], BF16) for i in range(_HG)], axis=1)
            y = jnp.dot(h_v[...], w, preferred_element_type=F32)
            pending.append((mg, y))
            return y[adv:seg, :]

        pending = []

        def flush():
            while pending:
                mg, y = pending.pop(0)
                for i, wp in enumerate(wpos):
                    ring[mg, pl.ds(wp, 8), :] = y[8 * i:8 * i + 8, :]

        def full(m, g, top):
            assert all(mg != m * n_grp + g for mg, _ in pending)
            return jnp.concatenate([top, ring[m * n_grp + g, pl.ds(rpos, seg), :]], axis=0)

        def probs(q, k):
            ps = []
            for i in range(_HG):
                sl = slice(i * Dh, (i + 1) * Dh)
                sc = jax.lax.dot_general(q[:, sl], k[:, sl], _NT, preferred_element_type=F32)
                sc = jnp.where(mask, sc * scale, _NEG)
                e = jnp.exp(sc - jnp.max(sc, axis=-1, keepdims=True))
                lsum = jnp.sum(e, axis=-1, keepdims=True)
                rc = pl.reciprocal(lsum, approx=True)
                rc = rc * (2.0 - lsum * rc)
                ps.append(e * rc)
            return ps

        def pv(ps, v, g):
            for i in range(_HG):
                sl = slice(i * Dh, (i + 1) * Dh)
                hh = g * _HG + i
                o_v[:, hh * Dh:(hh + 1) * Dh] = jnp.dot(ps[i], v[:, sl], preferred_element_type=F32)

        def oproj(g0, g1):
            k0, k1 = g0 * _HG * Dh, g1 * _HG * Dh
            w = jnp.concatenate([pltpu.bitcast(wo32[j, k0 // 2:k1 // 2, :], BF16)
                                 for j in range(n_dt)], axis=1)
            return jnp.dot(o_v[:, k0:k1], w, preferred_element_type=F32)

        top, p, acc = {}, {}, None
        for op in _order(CFG["order"]):
            if op[0] in "QKVC":
                flush()
            if op[0] in "QKV":
                m = "QKV".index(op[0])
                top[m, op[1]] = proj(m, op[1])
            elif op[0] == "S":
                g = op[1]
                p[g] = probs(full(0, g, top[0, g]), full(1, g, top[1, g]))
            elif op[0] == "P":
                g = op[1]
                pv(p[g], full(2, g, top[2, g]), g)
            else:
                part = oproj(op[1], op[2])
                acc = part if acc is None else acc + part

        flush()
        h_v[adv:seg, :] = _rb(acc[0:M, :])
        res = x_v[rows, :].astype(F32) + acc[M:L, :] * _silu(z_v[rows, :])
        out_v[rows, :] = res.astype(out_v.dtype)
        out_copy(s).start()
        return wrap(rd + seg // 8), wrap(wr_blk + adv // 8)

    if CFG["nsteps"]:
        n_seg = CFG["nsteps"]
    jax.lax.fori_loop(0, n_seg, step, (jnp.int32(0), jnp.int32(lead // 8)), unroll=CFG["unroll"])

    def drain(s, c):
        out_copy(s).wait()
        return c
    jax.lax.fori_loop(0, n_seg, drain, 0)


@functools.partial(jax.jit, static_argnames=("A_seg_len",))
def pallas_recurrent_scan__memory_aug_recurrent_mem_tr__moe_arch_mod__prompt_kernel(
    A_x, A_mem0, A_Wq, A_Wk, A_Wv, A_Wo, A_seg_len, B_x, B_w_r, B_w_gate, B_w_up, B_w_down,
):
    del B_x
    B, S, D = A_x.shape
    _, H, Dh = A_Wq.shape
    M = A_mem0.shape[1]
    Fh = B_w_gate.shape[1]
    seg = int(A_seg_len)
    L = M + seg
    n_dt = D // 128
    lead = (S // seg) * M
    n_chunk = 3 * H // _HC
    ring_rows = lead + seg

    hbm = pl.BlockSpec(memory_space=pltpu.MemorySpace.HBM)
    vmem = pl.BlockSpec(memory_space=pltpu.VMEM)
    out = pl.pallas_call(
        functools.partial(_kernel, seg=seg, n_heads=H, lead=lead, ln_rows0=640),
        out_shape=jax.ShapeDtypeStruct((S, D), A_x.dtype),
        in_specs=[hbm, vmem, hbm, hbm, hbm, hbm, vmem, hbm, hbm, hbm],
        out_specs=hbm,
        scratch_shapes=[
            pltpu.VMEM((S, D), A_x.dtype),
            pltpu.VMEM((lead, D), F32),
            pltpu.VMEM((S - lead, D), F32),
            pltpu.VMEM((S, D), F32),
            pltpu.VMEM((n_chunk, D * _HC // 2, Dh), U32),
            pltpu.VMEM((3 * H, D // 2, Dh), U32),
            pltpu.VMEM((3 * H // _HG, ring_rows, _HG * Dh), F32),
            pltpu.VMEM((n_dt, H * Dh, 128), BF16),
            pltpu.VMEM((Fh, D), BF16),
            pltpu.VMEM((Fh, D), BF16),
            pltpu.VMEM((Fh, D), BF16),
            pltpu.VMEM((seg, D), F32),
            pltpu.VMEM((L, H * Dh), F32),
            pltpu.VMEM((S, D), A_x.dtype),
            pltpu.SemaphoreType.DMA((5 + n_chunk + n_dt,)),
            pltpu.SemaphoreType.DMA((1,)),
        ],
        compiler_params=pltpu.CompilerParams(vmem_limit_bytes=110 * 1024 * 1024, flags=CFG.get("flags")),
        name="rmt_moe_scan",
    )(
        A_x.reshape(S, D),
        A_mem0.reshape(M, D),
        A_Wq,
        A_Wk,
        A_Wv,
        A_Wo.reshape(H * Dh, D),
        B_w_r,
        B_w_gate.T,
        B_w_up.T,
        B_w_down,
    )
    return out.reshape(B, S, D)
```

```python
import functools

import jax
import jax.numpy as jnp
import numpy as np
import jax.experimental.pallas as pl
import jax.experimental.pallas.tpu as pltpu

F32 = jnp.float32
BF16 = jnp.bfloat16
U32 = jnp.uint32

_TOPK = 8
_LN_EPS = 1e-5
_NEG = -1000000000.0
_HG = 4
_HC = 16
_NT = (((1,), (1,)), ((), ()))

CFG = dict(order="K0 Q0 K1 Q1 S0 V0 K2 Q2 S1 V1 P0 K3 Q3 S2 V2 P1 C0-1 K4 Q4 S3 V3 P2 C1-2 K5 Q5 S4 V4 P3 C2-3 K6 Q6 S5 V5 P4 C3-4 K7 Q7 S6 V6 S7 P5 C4-5 V7 P6 C5-6 P7 C6-7 C7-8",
           nsteps=None, unroll=8, prefetch='SP', ksplit=1, hbf16=1)


def _order(name):
    ops = []
    for tok in name.split():
        if tok[0] == "C":
            a, b = tok[1:].split("-")
            ops.append(("C", int(a), int(b)))
        else:
            ops.append((tok[0], int(tok[1:])))
    return ops


def _rb(v):
    return v.astype(BF16).astype(F32)


def _silu(v):
    return v * (1.0 / (1.0 + jnp.exp(-v)))


def _kernel(x_hbm, mem0_ref, wq_hbm, wk_hbm, wv_hbm, wo_hbm, wr_ref, wg_hbm, wu_hbm, wd_hbm,
            out_hbm,
            x_v, xa_v, xb_v, z_v, raw, w32, ring, wo_v, wg_v, wu_v, wd_v, h_v, h32_v, o_v, out_v,
            sems, sems0, semsx, out_sem, *, seg, n_heads, lead):
    n_chunk = raw.shape[0]
    n_grp = n_heads // _HG
    gpc = _HC // _HG
    S, D = x_v.shape
    M = mem0_ref.shape[0]
    L = M + seg
    n_seg = S // seg
    Dh = w32.shape[2]
    n_dt = D // 128
    scale = float(Dh) ** -0.5
    adv = seg - M
    ring_blk = ring.shape[1] // 8
    SKIP = CFG.get("skip_pro")

    n_it = 3 * n_grp
    pairs = _HC // 2
    gpi = CFG.get("gpi", 2)
    n_peel = 2
    n_loop = (n_it - gpc - n_peel) // gpi
    ln_first = 32
    ln_per = 80
    ln_rows0 = S - n_loop * gpi * ln_per
    xs = ln_rows0 + gpi * ln_per
    assert ln_rows0 <= lead + n_dt * ln_first <= xs
    lnb = 128

    def cp_xa(i):
        rows = pl.ds(pl.multiple_of(i * lnb, lnb), lnb)
        return pltpu.make_async_copy(x_hbm.at[rows, :], x_v.at[rows, :], semsx.at[i])

    cp_xm = pltpu.make_async_copy(x_hbm.at[lead:xs, :], x_v.at[lead:xs, :], sems.at[0])
    cp_xb = pltpu.make_async_copy(x_hbm.at[xs:S, :], x_v.at[xs:S, :], sems.at[1])

    def cp_w0(k):
        return pltpu.make_async_copy(
            wq_hbm.bitcast(U32).at[pl.ds(k * 128, 128), pl.ds(0, pairs), :],
            raw.at[0, pl.ds(pl.multiple_of(k * 128 * pairs, 128 * pairs), 128 * pairs), :]
            .reshape(128, pairs, Dh), sems0.at[k])

    cp_w = [None]
    for c in range(1, n_chunk):
        src = (wq_hbm, wk_hbm, wv_hbm)[c // (n_heads // _HC)].bitcast(U32)
        j0 = (c % (n_heads // _HC)) * pairs
        cp_w.append(pltpu.make_async_copy(src.at[:, pl.ds(j0, pairs), :],
                                          raw.at[c, pl.ds(0, D * pairs), :].reshape(D, pairs, Dh),
                                          sems.at[2 + c]))
    nb = 2 + n_chunk
    cp_o = [pltpu.make_async_copy(wo_hbm.at[:, pl.ds(j * 128, 128)], wo_v.at[j], sems.at[nb + j])
            for j in range(n_dt)]
    cp_g = pltpu.make_async_copy(wg_hbm, wg_v, sems.at[nb + n_dt])
    cp_u = pltpu.make_async_copy(wu_hbm, wu_v, sems.at[nb + n_dt + 1])
    cp_d = pltpu.make_async_copy(wd_hbm, wd_v, sems.at[nb + n_dt + 2])
    if not SKIP:
        def start_rows(i, c):
            cp_xa(i).start()
            return c
        jax.lax.fori_loop(0, lead // lnb, start_rows, 0)
        cp_xm.start()

        def start_slab(k, c):
            cp_w0(k).start()
            return c
        jax.lax.fori_loop(0, n_dt, start_slab, 0)
        for cp in [cp_w[1], cp_xb] + cp_w[2:] + [cp_g, cp_u, cp_d] + cp_o:
            cp.start()

    wr = wr_ref[...].astype(F32).reshape(1, D)
    eps = float(np.asarray(_LN_EPS, dtype=jnp.bfloat16).astype(np.float32))
    lane = jax.lax.broadcasted_iota(jnp.int32, (8, 128), 1)
    n_rv = S // (8 * 128)

    def ln_rows(row0, nrows, dst, dst0, racc):
        rows = pl.ds(row0, nrows)
        x32 = x_v[rows, :].astype(F32)
        mean = jnp.sum(x32, axis=-1, keepdims=True) * (1.0 / D)
        cen = x32 - mean
        var = jnp.sum(cen * cen, axis=-1, keepdims=True) * (1.0 / D)
        sd = _rb(jnp.sqrt(_rb(_rb(var) + eps)))
        xn = _rb(_rb(x32 - _rb(mean)) * (1.0 / sd))
        if dst.dtype == U32:
            packed = pltpu.bitcast(xn.astype(BF16), U32)
            for j in range(n_dt):
                dst[j, pl.ds(pl.multiple_of(dst0 // 2, 8), nrows // 2), :] = packed[:, j * 128:(j + 1) * 128]
        else:
            dst[pl.ds(dst0, nrows), :] = xn
        z_v[rows, :] = xn
        r = _rb(jnp.sum(xn * wr, axis=-1, keepdims=True))
        racc = list(racc)
        for b in range(nrows // 8):
            blk = row0 // 8 + b
            for j in range(n_rv):
                racc[j] = jnp.where(lane == blk - j * 128, r[b * 8:(b + 1) * 8, :], racc[j])
        return tuple(racc)

    def split_pair(a):
        return [pltpu.bitcast(half, U32) for half in (a.astype(jnp.uint16), (a >> 16).astype(jnp.uint16))]

    def first_step(k, racc):
        cp_w0(k).wait()
        cols = []
        for j in range(pairs):
            a = raw[0, pl.ds(k * 128 * pairs + j, 128, stride=pairs), :]
            for p, packed in enumerate(split_pair(a)):
                w32[2 * j + p, pl.ds(pl.multiple_of(k * 64, 64), 64), :] = packed
                cols.append(pltpu.bitcast(packed, BF16))
        xk = pltpu.bitcast(xa_v[k], BF16)
        for g in range(gpc):
            w = jnp.concatenate(cols[g * _HG:(g + 1) * _HG], axis=1)
            ring[g, 0:lead, :] += jnp.dot(xk, w, preferred_element_type=F32)
        off = pl.multiple_of(k * ln_first, ln_first)
        return ln_rows(lead + off, ln_first, xb_v, off, racc)

    def lead_group(it):
        c = it // gpc
        j0 = (it % gpc) * (_HG // 2)
        cols = []
        for jj in range(_HG // 2):
            a = raw[c, pl.ds(j0 + jj, D, stride=pairs), :]
            for p, packed in enumerate(split_pair(a)):
                w32[it * _HG + 2 * jj + p] = packed
                cols.append(pltpu.bitcast(packed, BF16))
        xa = jnp.concatenate([pltpu.bitcast(xa_v[j], BF16) for j in range(n_dt)], axis=1)
        ring[it, 0:lead, :] = jnp.dot(xa, jnp.concatenate(cols, axis=1), preferred_element_type=F32)

    def routing(racc):
        rr = jnp.concatenate(racc, axis=1) + 0.0
        tok = (jax.lax.broadcasted_iota(jnp.int32, rr.shape, 1) * 8
               + jax.lax.broadcasted_iota(jnp.int32, rr.shape, 0))
        bits = pltpu.bitcast(rr, jnp.int32)
        mono = jnp.where(bits < 0, bits ^ 0x7FFFFFFF, bits) >> 16
        key = pltpu.bitcast(0x30000000 + (mono + 32768) * S + (S - 1 - tok), F32)
        sub = jax.lax.broadcasted_iota(jnp.int32, (_TOPK, 1), 0)
        best = jnp.zeros((_TOPK, 1), F32)
        for i in range(_TOPK):
            m = jnp.max(jnp.max(key, axis=1, keepdims=True), axis=0, keepdims=True)
            key = jnp.where(key == m, 0.0, key)
            best = jnp.where(sub == i, m, best)
        kb = pltpu.bitcast(best, jnp.int32) - 0x30000000
        sel_tok = (S - 1) - (kb & (S - 1))
        mono = ((kb >> (S.bit_length() - 1)) - 32768) << 16
        r_sel = pltpu.bitcast(jnp.where(mono < 0, (mono | 0xFFFF) ^ 0x7FFFFFFF, mono), F32)
        idxs = [jnp.clip(jnp.max(jnp.where(sub == i, sel_tok, 0)), 0, S - 1) for i in range(_TOPK)]
        return idxs, r_sel, jnp.concatenate([z_v[pl.ds(ix, 1), :] for ix in idxs], axis=0)

    def expert(idxs, r_sel, x_sel):
        gp = _rb(jax.lax.dot_general(x_sel, wg_v[...], _NT, preferred_element_type=F32))
        up = _rb(jax.lax.dot_general(x_sel, wu_v[...], _NT, preferred_element_type=F32))
        gu = _rb(_rb(_silu(gp)) * up)
        y = _rb(jnp.dot(gu, wd_v[...], preferred_element_type=F32))
        y = _rb(y * _rb(1.0 / (1.0 + jnp.exp(-r_sel))))
        z_sel = _rb(x_sel + y)
        for i, ix in enumerate(idxs):
            z_v[pl.ds(ix, 1), :] = z_sel[i:i + 1, :]

    if not SKIP:
        ring[0:gpc, 0:lead, :] = jnp.zeros((gpc, lead, _HG * Dh), F32)
        racc = tuple(jnp.zeros((8, 128), F32) for _ in range(n_rv))

        def ln_lead(i, racc):
            cp_xa(i).wait()
            row0 = pl.multiple_of(i * lnb, lnb)
            return ln_rows(row0, lnb, xa_v, row0, racc)

        racc = jax.lax.fori_loop(0, lead // lnb, ln_lead, racc)
        cp_xm.wait()
        racc = jax.lax.fori_loop(0, n_dt, first_step, racc)

        def lead_step(it, racc):
            g0 = gpc + it * gpi

            @pl.when(g0 % gpc == 0)
            def _():
                chunk = raw.at[g0 // gpc, pl.ds(0, D * pairs), :]
                pltpu.make_async_copy(chunk, chunk, sems.at[2 + g0 // gpc]).wait()

            @pl.when(it == 1)
            def _():
                cp_xb.wait()

            PIN = CFG.get("pin")
            for u in range(gpi):
                lead_group(g0 + u)
                if PIN:
                    pieces = range(gpi) if u == 0 else ()
                else:
                    pieces = (u,)
                for v in pieces:
                    row0 = pl.multiple_of(ln_rows0 + (it * gpi + v) * ln_per, 16)
                    racc = ln_rows(row0, ln_per, xb_v, pl.multiple_of(row0 - lead, 16), racc)
                if PIN and u == 0:
                    xa_v[n_dt, pl.ds(pl.multiple_of(it * 8, 8), 8), :] = pltpu.bitcast(racc[0] + racc[1], U32)
            return racc

        racc = jax.lax.fori_loop(0, n_loop, lead_step, racc)
        cp_g.wait()
        cp_u.wait()
        cp_d.wait()
        routed = routing(racc)
        for u in range(n_it - n_peel, n_it - 1):
            lead_group(u)
        expert(*routed)
        lead_group(n_it - 1)
        for cp in cp_o:
            cp.wait()
    wo32 = wo_v.bitcast(U32)

    h_v[adv:seg, :] = mem0_ref[...].astype(F32)

    def out_copy(s):
        rows = pl.ds(pl.multiple_of(s * seg, seg), seg)
        return pltpu.make_async_copy(out_v.at[rows, :], out_hbm.at[rows, :], out_sem.at[0])

    def wrap(b):
        return jnp.where(b >= ring_blk, b - ring_blk, b)

    def step(s, carry):
        rd, wr_blk = carry
        rows = pl.ds(pl.multiple_of(s * seg, seg), seg)
        HB = CFG.get("hbf16")
        if HB:
            xr = xb_v[pl.ds(pl.multiple_of(s * adv, 8), adv), :]
            h32_v[0:8, :] = pltpu.bitcast(xr[0:16, :].astype(BF16), U32)
            h32_v[8:16, :] = pltpu.bitcast(
                jnp.concatenate([xr[16:adv, :], h_v[adv:seg, :]], axis=0).astype(BF16), U32)
        else:
            h_v[0:adv, :] = xb_v[pl.ds(pl.multiple_of(s * adv, 8), adv), :]

        def lhs(ks=slice(None)):
            return pltpu.bitcast(h32_v[:, ks], BF16) if HB else h_v[:, ks]
        ri = jax.lax.broadcasted_iota(jnp.int32, (L, L), 0)
        ci = jax.lax.broadcasted_iota(jnp.int32, (L, L), 1)
        mask = (ri < M) | (ri >= ci)
        wpos = [pl.multiple_of(wrap(wr_blk + i) * 8, 8) for i in range(adv // 8)]
        rpos = pl.multiple_of(rd * 8, seg)

        def proj(m, g, ksplit=False):
            mg = m * n_grp + g
            w = jnp.concatenate([pltpu.bitcast(w32[mg * _HG + i], BF16) for i in range(_HG)], axis=1)
            if ksplit:
                y = None
                for j in range(n_dt):
                    ks = slice(j * 128, (j + 1) * 128)
                    part = jnp.dot(lhs(ks), w[ks, :], preferred_element_type=F32)
                    y = part if y is None else y + part
            else:
                y = jnp.dot(lhs(), w, preferred_element_type=F32)
            pending.append((mg, y))
            return y[adv:seg, :]

        pending = []

        def flush():
            while pending:
                mg, y = pending.pop(0)
                for i, wp in enumerate(wpos):
                    ring[mg, pl.ds(wp, 8), :] = y[8 * i:8 * i + 8, :]

        seg_rows = {}

        def fetch(m, g):
            if (m, g) not in seg_rows:
                assert all(mg != m * n_grp + g for mg, _ in pending)
                seg_rows[m, g] = ring[m * n_grp + g, pl.ds(rpos, seg), :]

        def full(m, g, top):
            fetch(m, g)
            return jnp.concatenate([top, seg_rows[m, g]], axis=0)

        def probs(q, k):
            ps = []
            for i in range(_HG):
                sl = slice(i * Dh, (i + 1) * Dh)
                sc = jax.lax.dot_general(q[:, sl], k[:, sl], _NT, preferred_element_type=F32)
                sc = jnp.where(mask, sc * scale, _NEG)
                e = jnp.exp(sc - jnp.max(sc, axis=-1, keepdims=True))
                lsum = jnp.sum(e, axis=-1, keepdims=True)
                rc = pl.reciprocal(lsum, approx=True)
                rc = rc * (2.0 - lsum * rc)
                ps.append(e * rc)
            return ps

        def pv(ps, v, g):
            for i in range(_HG):
                sl = slice(i * Dh, (i + 1) * Dh)
                hh = g * _HG + i
                o_v[:, hh * Dh:(hh + 1) * Dh] = jnp.dot(ps[i], v[:, sl], preferred_element_type=F32)

        def oproj(g0, g1):
            k0, k1 = g0 * _HG * Dh, g1 * _HG * Dh
            w = jnp.concatenate([pltpu.bitcast(wo32[j, k0 // 2:k1 // 2, :], BF16)
                                 for j in range(n_dt)], axis=1)
            return jnp.dot(o_v[:, k0:k1], w, preferred_element_type=F32)

        top, p, acc = {}, {}, None
        ops = _order(CFG["order"])
        for n, op in enumerate(ops):
            if op[0] in "QKVC":
                for nxt in ops[n + 1:]:
                    if nxt[0] in "QKVC":
                        break
                    for m in {"S": (0, 1), "P": (2,)}[nxt[0]]:
                        ready = (m, nxt[1]) in top and all(mg != m * n_grp + nxt[1] for mg, _ in pending)
                        if ready and nxt[0] in CFG.get("prefetch", ""):
                            fetch(m, nxt[1])
                flush()
            if op[0] in "QKV":
                m = "QKV".index(op[0])
                top[m, op[1]] = proj(m, op[1], ksplit=(n == 0 and CFG.get("ksplit")))
            elif op[0] == "S":
                g = op[1]
                p[g] = probs(full(0, g, top[0, g]), full(1, g, top[1, g]))
            elif op[0] == "P":
                g = op[1]
                pv(p[g], full(2, g, top[2, g]), g)
            else:
                part = oproj(op[1], op[2])
                acc = part if acc is None else acc + part

        flush()
        h_v[adv:seg, :] = acc[0:M, :] if HB else _rb(acc[0:M, :])
        res = x_v[rows, :].astype(F32) + acc[M:L, :] * _silu(z_v[rows, :])
        out_v[rows, :] = res.astype(out_v.dtype)
        out_copy(s).start()
        return wrap(rd + seg // 8), wrap(wr_blk + adv // 8)

    if CFG["nsteps"]:
        n_seg = CFG["nsteps"]
    jax.lax.fori_loop(0, n_seg, step, (jnp.int32(0), jnp.int32(lead // 8)), unroll=CFG["unroll"])

    def drain(s, c):
        out_copy(s).wait()
        return c
    jax.lax.fori_loop(0, n_seg, drain, 0)


@functools.partial(jax.jit, static_argnames=("A_seg_len",))
def pallas_recurrent_scan__memory_aug_recurrent_mem_tr__moe_arch_mod__prompt_kernel(
    A_x, A_mem0, A_Wq, A_Wk, A_Wv, A_Wo, A_seg_len, B_x, B_w_r, B_w_gate, B_w_up, B_w_down,
):
    del B_x
    B, S, D = A_x.shape
    _, H, Dh = A_Wq.shape
    M = A_mem0.shape[1]
    Fh = B_w_gate.shape[1]
    seg = int(A_seg_len)
    L = M + seg
    n_dt = D // 128
    lead = (S // seg) * M
    n_chunk = 3 * H // _HC
    ring_rows = lead + seg

    hbm = pl.BlockSpec(memory_space=pltpu.MemorySpace.HBM)
    vmem = pl.BlockSpec(memory_space=pltpu.VMEM)
    out = pl.pallas_call(
        functools.partial(_kernel, seg=seg, n_heads=H, lead=lead),
        out_shape=jax.ShapeDtypeStruct((S, D), A_x.dtype),
        in_specs=[hbm, vmem, hbm, hbm, hbm, hbm, vmem, hbm, hbm, hbm],
        out_specs=hbm,
        scratch_shapes=[
            pltpu.VMEM((S, D), A_x.dtype),
            pltpu.VMEM((n_dt + 1, lead // 2, 128), U32),
            pltpu.VMEM((S - lead, D), F32),
            pltpu.VMEM((S, D), F32),
            pltpu.VMEM((n_chunk, D * _HC // 2 + 8, Dh), U32),
            pltpu.VMEM((3 * H, D // 2, Dh), U32),
            pltpu.VMEM((3 * H // _HG, ring_rows, _HG * Dh), F32),
            pltpu.VMEM((n_dt, H * Dh, 128), BF16),
            pltpu.VMEM((Fh, D), BF16),
            pltpu.VMEM((Fh, D), BF16),
            pltpu.VMEM((Fh, D), BF16),
            pltpu.VMEM((seg, D), F32),
            pltpu.VMEM((seg // 2, D), U32),
            pltpu.VMEM((L, H * Dh), F32),
            pltpu.VMEM((S, D), A_x.dtype),
            pltpu.SemaphoreType.DMA((5 + n_chunk + n_dt,)),
            pltpu.SemaphoreType.DMA((n_dt,)),
            pltpu.SemaphoreType.DMA((lead // 128,)),
            pltpu.SemaphoreType.DMA((1,)),
        ],
        compiler_params=pltpu.CompilerParams(vmem_limit_bytes=110 * 1024 * 1024, flags=CFG.get("flags")),
        name="rmt_moe_scan",
    )(
        A_x.reshape(S, D),
        A_mem0.reshape(M, D),
        A_Wq,
        A_Wk,
        A_Wv,
        A_Wo.reshape(H * Dh, D),
        B_w_r,
        B_w_gate.T,
        B_w_up.T,
        B_w_down,
    )
    return out.reshape(B, S, D)
```

```python
import functools

import jax
import jax.numpy as jnp
import numpy as np
import jax.experimental.pallas as pl
import jax.experimental.pallas.tpu as pltpu

F32 = jnp.float32
BF16 = jnp.bfloat16
U32 = jnp.uint32

_TOPK = 8
_LN_EPS = 1e-5
_MASKED = -1000000000.0
_LANES = 128
_HG = 4
_HC = 16
_PAIRS = _HC // 2
_SLAB = _LANES * _PAIRS + 8
_X_ROWS = 128
_LN_FIRST = 32
_LN_LEAD = 80
_GROUPS_PER_ITER = 2
_SCAN_UNROLL = 8
_NT = (((1,), (1,)), ((), ()))

_STEP_ORDER = (
    "K0 Q0 K1 Q1 S0 V0 K2 Q2 S1 V1 P0 K3 Q3 S2 V2 P1 C0 K4 Q4 S3 V3 P2 C1 "
    "K5 Q5 S4 V4 P3 C2 K6 Q6 S5 V5 P4 C3 K7 Q7 S6 V6 S7 P5 C4 V7 P6 C5 P7 C6 C7"
)


def _rb(v):
    return v.astype(BF16).astype(F32)


def _sigmoid(v):
    return 1.0 / (1.0 + jnp.exp(-v))


def _silu(v):
    return v * _sigmoid(v)


def _split_pair(a):
    return [pltpu.bitcast(half, U32)
            for half in (a.astype(jnp.uint16), (a >> 16).astype(jnp.uint16))]


def _kernel(x_hbm, mem0_ref, wq_hbm, wk_hbm, wv_hbm, wo_hbm, wr_ref, wg_hbm, wu_hbm, wd_hbm,
            out_hbm,
            x_v, xa_v, xb_v, z_v, raw, w32, ring, wo_v, wg_v, wu_v, wd_v, mem_v, h_v, o_v, out_v,
            sems, slab_sems, x_sems, out_sem, *, seg, n_heads, lead):
    S, D = x_v.shape
    M = mem0_ref.shape[0]
    Dh = w32.shape[2]
    L = M + seg
    n_seg = S // seg
    n_dt = D // _LANES
    n_grp = n_heads // _HG
    n_all = 3 * n_grp
    n_chunk = raw.shape[0]
    gpc = _HC // _HG
    adv = seg - M
    ring_blk = ring.shape[1] // 8
    scale = float(Dh) ** -0.5
    n_loop = (n_all - gpc - 2) // _GROUPS_PER_ITER
    ln_start = S - n_loop * _GROUPS_PER_ITER * _LN_LEAD
    x_mid = ln_start + _GROUPS_PER_ITER * _LN_LEAD
    assert lead <= ln_start <= lead + n_dt * _LN_FIRST <= x_mid and ln_start % 16 == 0

    def cp_x_lead(i):
        rows = pl.ds(pl.multiple_of(i * _X_ROWS, _X_ROWS), _X_ROWS)
        return pltpu.make_async_copy(x_hbm.at[rows, :], x_v.at[rows, :], x_sems.at[i])

    def cp_slab(k):
        dst = raw.at[0, pl.ds(pl.multiple_of(k * _SLAB, 8), _LANES * _PAIRS), :]
        return pltpu.make_async_copy(
            wq_hbm.bitcast(U32).at[pl.ds(k * _LANES, _LANES), pl.ds(0, _PAIRS), :],
            dst.reshape(_LANES, _PAIRS, Dh), slab_sems.at[k])

    cp_x_mid = pltpu.make_async_copy(x_hbm.at[lead:x_mid, :], x_v.at[lead:x_mid, :], sems.at[0])
    cp_x_rest = pltpu.make_async_copy(x_hbm.at[x_mid:S, :], x_v.at[x_mid:S, :], sems.at[1])
    cp_chunk = {}
    for c in range(1, n_chunk):
        src = (wq_hbm, wk_hbm, wv_hbm)[c // (n_heads // _HC)].bitcast(U32)
        cp_chunk[c] = pltpu.make_async_copy(
            src.at[:, pl.ds((c % (n_heads // _HC)) * _PAIRS, _PAIRS), :],
            raw.at[c, pl.ds(0, D * _PAIRS), :].reshape(D, _PAIRS, Dh), sems.at[1 + c])
    nb = 1 + n_chunk
    cp_ffn = [pltpu.make_async_copy(src, dst, sems.at[nb + i])
              for i, (src, dst) in enumerate(((wg_hbm, wg_v), (wu_hbm, wu_v), (wd_hbm, wd_v)))]
    cp_wo = [pltpu.make_async_copy(wo_hbm.at[:, pl.ds(j * _LANES, _LANES)], wo_v.at[j],
                                   sems.at[nb + 3 + j]) for j in range(n_dt)]

    def start_all(copy, n):
        def body(i, carry):
            copy(i).start()
            return carry
        jax.lax.fori_loop(0, n, body, 0)

    start_all(cp_x_lead, lead // _X_ROWS)
    cp_x_mid.start()
    start_all(cp_slab, n_dt)
    for cp in [cp_chunk[1], cp_x_rest] + [cp_chunk[c] for c in range(2, n_chunk)] + cp_ffn + cp_wo:
        cp.start()

    w_r = wr_ref[...].astype(F32).reshape(1, D)
    eps = float(np.asarray(_LN_EPS, dtype=jnp.bfloat16).astype(np.float32))
    lane = jax.lax.broadcasted_iota(jnp.int32, (8, _LANES), 1)
    n_rv = S // (8 * _LANES)

    def layernorm(row0, nrows, scores):
        rows = pl.ds(row0, nrows)
        x32 = x_v[rows, :].astype(F32)
        mean = jnp.sum(x32, axis=-1, keepdims=True) * (1.0 / D)
        cen = x32 - mean
        var = jnp.sum(cen * cen, axis=-1, keepdims=True) * (1.0 / D)
        sd = _rb(jnp.sqrt(_rb(_rb(var) + eps)))
        xn = _rb(_rb(x32 - _rb(mean)) * (1.0 / sd))
        z_v[rows, :] = xn
        r = _rb(jnp.sum(xn * w_r, axis=-1, keepdims=True))
        scores = list(scores)
        for b in range(nrows // 8):
            blk = row0 // 8 + b
            for j in range(n_rv):
                scores[j] = jnp.where(lane == blk - j * _LANES, r[b * 8:(b + 1) * 8, :], scores[j])
        return xn, tuple(scores)

    def layernorm_rest(row0, nrows, scores):
        xn, scores = layernorm(row0, nrows, scores)
        xb_v[pl.ds(pl.multiple_of(row0 - lead, 16), nrows), :] = xn
        return scores

    def layernorm_lead(i, scores):
        cp_x_lead(i).wait()
        xn, scores = layernorm(pl.multiple_of(i * _X_ROWS, _X_ROWS), _X_ROWS, scores)
        packed = pltpu.bitcast(xn.astype(BF16), U32)
        rows = pl.ds(pl.multiple_of(i * (_X_ROWS // 2), _X_ROWS // 2), _X_ROWS // 2)
        for j in range(n_dt):
            xa_v[j, rows, :] = packed[:, j * _LANES:(j + 1) * _LANES]
        return scores

    def first_chunk_slab(k, scores):
        cp_slab(k).wait()
        cols = []
        for j in range(_PAIRS):
            a = raw[0, pl.ds(k * _SLAB + j, _LANES, stride=_PAIRS), :]
            for p, packed in enumerate(_split_pair(a)):
                rows = pl.ds(pl.multiple_of(k * (_LANES // 2), _LANES // 2), _LANES // 2)
                w32[2 * j + p, rows, :] = packed
                cols.append(pltpu.bitcast(packed, BF16))
        xk = pltpu.bitcast(xa_v[k], BF16)
        for g in range(gpc):
            w = jnp.concatenate(cols[g * _HG:(g + 1) * _HG], axis=1)
            ring[g, 0:lead, :] += jnp.dot(xk, w, preferred_element_type=F32)
        return layernorm_rest(pl.multiple_of(lead + k * _LN_FIRST, 16), _LN_FIRST, scores)

    def lead_group(g):
        cols = []
        for jj in range(_HG // 2):
            a = raw[g // gpc, pl.ds((g % gpc) * (_HG // 2) + jj, D, stride=_PAIRS), :]
            for p, packed in enumerate(_split_pair(a)):
                w32[g * _HG + 2 * jj + p] = packed
                cols.append(pltpu.bitcast(packed, BF16))
        xa = jnp.concatenate([pltpu.bitcast(xa_v[j], BF16) for j in range(n_dt)], axis=1)
        ring[g, 0:lead, :] = jnp.dot(xa, jnp.concatenate(cols, axis=1), preferred_element_type=F32)

    def lead_groups(it, scores):
        g0 = gpc + it * _GROUPS_PER_ITER

        @pl.when(g0 % gpc == 0)
        def _():
            chunk = raw.at[g0 // gpc, pl.ds(0, D * _PAIRS), :]
            pltpu.make_async_copy(chunk, chunk, sems.at[1 + g0 // gpc]).wait()

        @pl.when(it == 1)
        def _():
            cp_x_rest.wait()

        for u in range(_GROUPS_PER_ITER):
            lead_group(g0 + u)
            row0 = ln_start + (it * _GROUPS_PER_ITER + u) * _LN_LEAD
            scores = layernorm_rest(pl.multiple_of(row0, 16), _LN_LEAD, scores)
            if u + 1 < _GROUPS_PER_ITER:
                spare = pl.ds(pl.multiple_of(it * 8, 8), 8)
                xa_v[n_dt, spare, :] = pltpu.bitcast(sum(scores[1:], scores[0]), U32)
        return scores

    def route(scores):
        r = jnp.concatenate(scores, axis=1) + 0.0
        tok = (jax.lax.broadcasted_iota(jnp.int32, r.shape, 1) * 8
               + jax.lax.broadcasted_iota(jnp.int32, r.shape, 0))
        bits = pltpu.bitcast(r, jnp.int32)
        mono = jnp.where(bits < 0, bits ^ 0x7FFFFFFF, bits) >> 16
        key = pltpu.bitcast(0x30000000 + (mono + 32768) * S + (S - 1 - tok), F32)
        slot = jax.lax.broadcasted_iota(jnp.int32, (_TOPK, 1), 0)
        best = jnp.zeros((_TOPK, 1), F32)
        for i in range(_TOPK):
            m = jnp.max(jnp.max(key, axis=1, keepdims=True), axis=0, keepdims=True)
            key = jnp.where(key == m, 0.0, key)
            best = jnp.where(slot == i, m, best)
        kb = pltpu.bitcast(best, jnp.int32) - 0x30000000
        sel_tok = (S - 1) - (kb & (S - 1))
        mono = ((kb >> (S.bit_length() - 1)) - 32768) << 16
        r_sel = pltpu.bitcast(jnp.where(mono < 0, (mono | 0xFFFF) ^ 0x7FFFFFFF, mono), F32)
        idx = [jnp.clip(jnp.max(jnp.where(slot == i, sel_tok, 0)), 0, S - 1)
               for i in range(_TOPK)]
        return idx, r_sel, jnp.concatenate([z_v[pl.ds(t, 1), :] for t in idx], axis=0)

    def expert(idx, r_sel, x_sel):
        gate = _rb(jax.lax.dot_general(x_sel, wg_v[...], _NT, preferred_element_type=F32))
        up = _rb(jax.lax.dot_general(x_sel, wu_v[...], _NT, preferred_element_type=F32))
        y = _rb(jnp.dot(_rb(_rb(_silu(gate)) * up), wd_v[...], preferred_element_type=F32))
        z_sel = _rb(x_sel + _rb(y * _rb(_sigmoid(r_sel))))
        for i, t in enumerate(idx):
            z_v[pl.ds(t, 1), :] = z_sel[i:i + 1, :]

    ring[0:gpc, 0:lead, :] = jnp.zeros((gpc, lead, _HG * Dh), F32)
    scores = tuple(jnp.zeros((8, _LANES), F32) for _ in range(n_rv))
    scores = jax.lax.fori_loop(0, lead // _X_ROWS, layernorm_lead, scores)
    cp_x_mid.wait()
    scores = jax.lax.fori_loop(0, n_dt, first_chunk_slab, scores)
    scores = jax.lax.fori_loop(0, n_loop, lead_groups, scores)
    for cp in cp_ffn:
        cp.wait()
    routed = route(scores)
    lead_group(n_all - 2)
    expert(*routed)
    lead_group(n_all - 1)
    for cp in cp_wo:
        cp.wait()

    wo32 = wo_v.bitcast(U32)
    mem_v[...] = mem0_ref[...].astype(F32)
    order = [(tok[0], int(tok[1:])) for tok in _STEP_ORDER.split()]

    def cp_out(s):
        rows = pl.ds(pl.multiple_of(s * seg, seg), seg)
        return pltpu.make_async_copy(out_v.at[rows, :], out_hbm.at[rows, :], out_sem.at[0])

    def wrap(blk):
        return jnp.where(blk >= ring_blk, blk - ring_blk, blk)

    def step(s, carry):
        rd, wr = carry
        rows = pl.ds(pl.multiple_of(s * seg, seg), seg)
        rd_rows = pl.ds(pl.multiple_of(rd * 8, seg), seg)
        wr_rows = [pl.ds(pl.multiple_of(wrap(wr + i) * 8, 8), 8) for i in range(adv // 8)]

        xr = xb_v[pl.ds(pl.multiple_of(s * adv, 8), adv), :]
        h_v[0:8, :] = pltpu.bitcast(xr[0:16, :].astype(BF16), U32)
        h_v[8:16, :] = pltpu.bitcast(
            jnp.concatenate([xr[16:adv, :], mem_v[...]], axis=0).astype(BF16), U32)

        qi = jax.lax.broadcasted_iota(jnp.int32, (L, L), 0)
        ki = jax.lax.broadcasted_iota(jnp.int32, (L, L), 1)
        mask = (qi < M) | (qi >= ki)

        mem_rows, seg_rows, probs = {}, {}, {}
        pending = []

        def flush():
            while pending:
                g, y = pending.pop(0)
                for i, dst in enumerate(wr_rows):
                    ring[g, dst, :] = y[8 * i:8 * i + 8, :]

        def fetch(g):
            if g not in seg_rows:
                assert all(g != pg for pg, _ in pending)
                seg_rows[g] = ring[g, rd_rows, :]

        def project(g, by_slab):
            w = jnp.concatenate([pltpu.bitcast(w32[g * _HG + i], BF16) for i in range(_HG)], axis=1)
            if by_slab:
                y = None
                for j in range(n_dt):
                    ks = slice(j * _LANES, (j + 1) * _LANES)
                    part = jnp.dot(pltpu.bitcast(h_v[:, ks], BF16), w[ks, :],
                                   preferred_element_type=F32)
                    y = part if y is None else y + part
            else:
                y = jnp.dot(pltpu.bitcast(h_v[...], BF16), w, preferred_element_type=F32)
            pending.append((g, y))
            mem_rows[g] = y[adv:seg, :]

        def operand(g):
            fetch(g)
            return jnp.concatenate([mem_rows[g], seg_rows[g]], axis=0)

        def softmax_scores(q, k):
            ps = []
            for i in range(_HG):
                hs = slice(i * Dh, (i + 1) * Dh)
                sc = jax.lax.dot_general(q[:, hs], k[:, hs], _NT, preferred_element_type=F32)
                sc = jnp.where(mask, sc * scale, _MASKED)
                e = jnp.exp(sc - jnp.max(sc, axis=-1, keepdims=True))
                den = jnp.sum(e, axis=-1, keepdims=True)
                inv = pl.reciprocal(den, approx=True)
                ps.append(e * (inv * (2.0 - den * inv)))
            return ps

        def attend(ps, v, g):
            for i in range(_HG):
                head = g * _HG + i
                o_v[:, head * Dh:(head + 1) * Dh] = jnp.dot(
                    ps[i], v[:, i * Dh:(i + 1) * Dh], preferred_element_type=F32)

        def out_project(g):
            k0, k1 = g * _HG * Dh, (g + 1) * _HG * Dh
            w = jnp.concatenate([pltpu.bitcast(wo32[j, k0 // 2:k1 // 2, :], BF16)
                                 for j in range(n_dt)], axis=1)
            return jnp.dot(o_v[:, k0:k1], w, preferred_element_type=F32)

        ring_groups = {"S": (0, n_grp), "P": (2 * n_grp,)}
        acc = None
        for n, (op, g) in enumerate(order):
            if op in "QKVC":
                for nop, ng in order[n + 1:]:
                    if nop in "QKVC":
                        break
                    for base in ring_groups[nop]:
                        if base + ng in mem_rows and all(base + ng != pg for pg, _ in pending):
                            fetch(base + ng)
                flush()
            if op in "QKV":
                project("QKV".index(op) * n_grp + g, by_slab=(n == 0))
            elif op == "S":
                probs[g] = softmax_scores(operand(g), operand(n_grp + g))
            elif op == "P":
                attend(probs[g], operand(2 * n_grp + g), g)
            else:
                part = out_project(g)
                acc = part if acc is None else acc + part
        flush()

        mem_v[...] = acc[0:M, :]
        res = x_v[rows, :].astype(F32) + acc[M:L, :] * _silu(z_v[rows, :])
        out_v[rows, :] = res.astype(out_v.dtype)
        cp_out(s).start()
        return wrap(rd + seg // 8), wrap(wr + adv // 8)

    jax.lax.fori_loop(0, n_seg, step, (jnp.int32(0), jnp.int32(lead // 8)), unroll=_SCAN_UNROLL)

    def drain(s, carry):
        cp_out(s).wait()
        return carry
    jax.lax.fori_loop(0, n_seg, drain, 0)


@functools.partial(jax.jit, static_argnames=("A_seg_len",))
def pallas_recurrent_scan__memory_aug_recurrent_mem_tr__moe_arch_mod__prompt_kernel(
    A_x: jax.Array,
    A_mem0: jax.Array,
    A_Wq: jax.Array,
    A_Wk: jax.Array,
    A_Wv: jax.Array,
    A_Wo: jax.Array,
    A_seg_len: int,
    B_x: jax.Array,
    B_w_r: jax.Array,
    B_w_gate: jax.Array,
    B_w_up: jax.Array,
    B_w_down: jax.Array,
):
    del B_x
    B, S, D = A_x.shape
    _, H, Dh = A_Wq.shape
    M = A_mem0.shape[1]
    Fh = B_w_gate.shape[1]
    seg = int(A_seg_len)
    assert (B, H, Dh, M, seg) == (1, 32, _LANES, 8, 32) and D % _LANES == 0
    assert S % (8 * _LANES) == 0 and S & (S - 1) == 0
    n_dt = D // _LANES
    n_chunk = 3 * H // _HC
    lead = (S // seg) * M

    hbm = pl.BlockSpec(memory_space=pltpu.MemorySpace.HBM)
    vmem = pl.BlockSpec(memory_space=pltpu.VMEM)
    out = pl.pallas_call(
        functools.partial(_kernel, seg=seg, n_heads=H, lead=lead),
        out_shape=jax.ShapeDtypeStruct((S, D), A_x.dtype),
        in_specs=[hbm, vmem, hbm, hbm, hbm, hbm, vmem, hbm, hbm, hbm],
        out_specs=hbm,
        scratch_shapes=[
            pltpu.VMEM((S, D), A_x.dtype),
            pltpu.VMEM((n_dt + 1, lead // 2, _LANES), U32),
            pltpu.VMEM((S - lead, D), F32),
            pltpu.VMEM((S, D), F32),
            pltpu.VMEM((n_chunk, n_dt * _SLAB, Dh), U32),
            pltpu.VMEM((3 * H, D // 2, Dh), U32),
            pltpu.VMEM((3 * H // _HG, lead + seg, _HG * Dh), F32),
            pltpu.VMEM((n_dt, H * Dh, _LANES), BF16),
            pltpu.VMEM((Fh, D), BF16),
            pltpu.VMEM((Fh, D), BF16),
            pltpu.VMEM((Fh, D), BF16),
            pltpu.VMEM((M, D), F32),
            pltpu.VMEM((seg // 2, D), U32),
            pltpu.VMEM((M + seg, H * Dh), F32),
            pltpu.VMEM((S, D), A_x.dtype),
            pltpu.SemaphoreType.DMA((4 + n_chunk + n_dt,)),
            pltpu.SemaphoreType.DMA((n_dt,)),
            pltpu.SemaphoreType.DMA((lead // _X_ROWS,)),
            pltpu.SemaphoreType.DMA((1,)),
        ],
        compiler_params=pltpu.CompilerParams(vmem_limit_bytes=110 * 1024 * 1024),
        name="rmt_moe_scan",
    )(
        A_x.reshape(S, D),
        A_mem0.reshape(M, D),
        A_Wq,
        A_Wk,
        A_Wv,
        A_Wo.reshape(H * Dh, D),
        B_w_r,
        B_w_gate.T,
        B_w_up.T,
        B_w_down,
    )
    return out.reshape(B, S, D)
```
